```python
import os as _os
_os.environ.setdefault("JAX_PLATFORMS", "cpu")
import jax
import jax.numpy as jnp

def _softmax(x, axis=-1):
    return jax.nn.softmax(x, axis=axis)
def _gelu(x):
    return jax.nn.gelu(x, approximate=True)
def _silu(x):
    return jax.nn.silu(x)
def _sigmoid(x):
    return jax.nn.sigmoid(x)
def _layernorm(x, axis=-1, eps=1e-5):
    m = jnp.mean(x, axis=axis, keepdims=True)
    v = jnp.var(x, axis=axis, keepdims=True)
    return (x - m) / jnp.sqrt(v + eps)
def _scatter_add(tgt, idx, src, axis=0):
    return tgt.at[idx].add(src)
def _segment_sum(src, seg, n):
    return jax.ops.segment_sum(src, seg, n)
class _Rng:
    def __init__(self, key):
        self._k = key
    def _next(self):
        self._k, sub = jax.random.split(self._k)
        return sub
    def normal(self, shape):
        return jax.random.normal(self._next(), shape, dtype=jnp.bfloat16)
    def randint(self, lo, hi, shape):
        return jax.random.randint(self._next(), shape, lo, hi, dtype=jnp.int32)
    def uniform(self, shape, lo=0.0, hi=1.0):
        return jax.random.uniform(self._next(), shape, jnp.bfloat16, lo, hi)
    def permutation(self, n):
        return jax.random.permutation(self._next(), n)


kernel_name = 'sequential_preLN__sliding_local_dilated__dense_activation_mish__prompt'

def setup_inputs():
    _rng = _Rng(jax.random.key(int.from_bytes(__import__("os").urandom(4), "little")))
    _w = (lambda a: (lambda t: t.astype(jnp.bfloat16) if jnp.issubdtype(t.dtype, jnp.floating) else t)(jnp.asarray(a)))
    def _A_setup():
        B, S, D = 1, 2048, 512
        return {
            "x": _w((lambda *s: _rng.normal(s) * 0.05)(B, S, D)),
            "wqkv": _w((lambda *s: _rng.normal(s) * 0.05)(D, 3 * D)),
            "wo": _w((lambda *s: _rng.normal(s) * 0.05)(D, D)),
        }
    _A_in = _A_setup()

    def _B_setup():
        B, S, D, F = 1, 2048, 512, 1376
        return {
            "x": _w((lambda *s: _rng.normal(s) * 0.05)(B, S, D)),
            "w1": _w((lambda *s: _rng.normal(s) * 1.6)(D, F) * (D ** -0.5)),
            "b1": _w((lambda *s: _rng.normal(s) * 0.1)(F)),
            "w2": _w((lambda *s: _rng.normal(s) * 0.1)(F, D) * (F ** -0.5)),
        }
    _B_in = _B_setup()

    return {
        "A_x": _A_in["x"],
        "A_wqkv": _A_in["wqkv"],
        "A_wo": _A_in["wo"],
        "B_x": _B_in["x"],
        "B_w1": _B_in["w1"],
        "B_b1": _B_in["b1"],
        "B_w2": _B_in["w2"],
    }

def reference(A_x, A_wqkv, A_wo, B_x, B_w1, B_b1, B_w2):
    def _A_ref(x, wqkv, wo):
        B, S, D = x.shape
        H = 32; Dh = D // H
        W, dil = 8, 2
        qkv = (lambda x, *d: x.transpose(*d))((x @ wqkv).reshape(B, S, 3, H, Dh), 2, 0, 3, 1, 4)
        q, k, v = qkv[0], qkv[1], qkv[2]
        scale = Dh ** -0.5
        pos = jnp.arange(S)
        off = jnp.arange(W) * dil
        idx = pos[:, None] - off[None, :]
        mask = idx >= 0
        idx_c = jnp.where(mask, idx, 0).reshape(-1)
        kg = k[:, :, idx_c, :].reshape(B, H, S, W, Dh)
        vg = v[:, :, idx_c, :].reshape(B, H, S, W, Dh)
        logits = jnp.einsum("bhsd,bhswd->bhsw", q, kg) * scale
        logits = jnp.where(mask[None, None, :, :], logits, -1e9)
        attn = _softmax(logits, axis=-1)
        o = jnp.einsum("bhsw,bhswd->bhsd", attn, vg)
        return (lambda x, *d: x.transpose(*d))(o, 0, 2, 1, 3).reshape(B, S, D) @ wo

    def _B_ref(x, w1, b1, w2):
        h = jnp.einsum("bsd,df->bsf", x, w1) + b1
        sp = jnp.log1p(jnp.exp(-jnp.abs(h))) + jnp.where(h > 0, h, jnp.zeros_like(h))
        act = h * jnp.tanh(sp)
        return jnp.einsum("bsf,fd->bsd", act, w2)

    x = A_x
    h = x + _A_ref(_layernorm(x, axis=-1), A_wqkv, A_wo)
    h2 = h + _B_ref(_layernorm(h, axis=-1), B_w1, B_b1, B_w2)
    return h2
```

```python
import functools

import jax
import jax.numpy as jnp
import jax.experimental.pallas as pl
import jax.experimental.pallas.tpu as pltpu

H = 32
W = 8
DIL = 2
HALO = 16
EPS = 1e-5
LANES = 128


def _layernorm(x):
    m = jnp.mean(x, axis=-1, keepdims=True)
    xc = x - m
    v = jnp.mean(xc * xc, axis=-1, keepdims=True)
    return xc * jax.lax.rsqrt(v + EPS)


def _kernel(x0_ref, x1_ref, x2_ref, wqkv_hbm, wo_hbm, w1t_hbm, b1_ref, w2_hbm, o_ref,
            wqkv_s, wo_s, w1t_s, w2_s, wqkv_p, wo_p, w1_s, kv_scr, h_scr, xn_scr, sems,
            *, tb, d, nblk):
    i = pl.program_id(0)
    dh = d // H
    scale = dh ** -0.5
    nt = d // LANES

    def ln1(x_ref):
        return _layernorm(x_ref[...].astype(jnp.float32)).astype(jnp.bfloat16)

    def attention(xn, blk):
        qkv = jnp.dot(xn, wqkv_p[...], preferred_element_type=jnp.float32)
        q = qkv[:, :d] * scale
        kv_scr[HALO:HALO + tb, :] = qkv[:, d:]
        row = blk * tb + jax.lax.broadcasted_iota(jnp.int32, (tb, LANES), 0)
        logits = []
        for w in range(W):
            kw = kv_scr[pl.ds(HALO - DIL * w, tb), 0:d]
            p = q * kw
            s = p[:, 0:LANES]
            for c in range(1, nt):
                s = s + p[:, c * LANES:(c + 1) * LANES]
            s = s + pltpu.roll(s, 64, 1)
            s = s + pltpu.roll(s, 32, 1)
            logits.append(jnp.where(row >= DIL * w, s, -1e9))
        m = logits[0]
        for w in range(1, W):
            m = jnp.maximum(m, logits[w])
        es = [jnp.exp(l - m) for l in logits]
        den = es[0]
        for w in range(1, W):
            den = den + es[w]
        inv = 1.0 / den
        o = None
        for w in range(W):
            vw = kv_scr[pl.ds(HALO - DIL * w, tb), d:2 * d]
            a = es[w] * inv
            a = jnp.concatenate([a] * nt, axis=1)
            t = a * vw
            o = t if o is None else o + t
        kv_scr[0:HALO, :] = kv_scr[tb:tb + HALO, :]
        return o

    def attention2(x_ref, o):
        attn = jnp.dot(o.astype(jnp.bfloat16), wo_p[...], preferred_element_type=jnp.float32)
        h_scr[...] = x_ref[...].astype(jnp.float32) + attn

    def ln2():
        return _layernorm(h_scr[...]).astype(jnp.bfloat16)

    def ffn(hn):
        z = jnp.dot(hn, w1_s[...], preferred_element_type=jnp.float32)
        z = z + b1_ref[...].astype(jnp.float32)
        sp = jnp.log1p(jnp.exp(-jnp.abs(z))) + jnp.maximum(z, 0.0)
        act = z * jnp.tanh(sp)
        y = jnp.dot(act.astype(jnp.bfloat16), w2_s[...], preferred_element_type=jnp.float32)
        o_ref[...] = (h_scr[...] + y).astype(o_ref.dtype)

    @pl.when(i == 0)
    def _():
        cps = [
            pltpu.make_async_copy(wqkv_hbm, wqkv_s, sems.at[0]),
            pltpu.make_async_copy(wo_hbm, wo_s, sems.at[1]),
            pltpu.make_async_copy(w1t_hbm, w1t_s, sems.at[2]),
            pltpu.make_async_copy(w2_hbm, w2_s, sems.at[3]),
        ]
        for cp in cps:
            cp.start()
        kv_scr[0:HALO, :] = jnp.zeros((HALO, 2 * d), jnp.float32)
        r = jax.lax.broadcasted_iota(jnp.int32, (d, d), 0)
        c = jax.lax.broadcasted_iota(jnp.int32, (d, d), 1)
        perm = (c == (r % dh) * H + r // dh).astype(jnp.bfloat16)
        perm_t = (r == (c % dh) * H + c // dh).astype(jnp.bfloat16)
        cps[0].wait()
        for j in range(3):
            wqkv_p[:, j * d:(j + 1) * d] = jnp.dot(
                wqkv_s[:, j * d:(j + 1) * d], perm,
                preferred_element_type=jnp.float32).astype(jnp.bfloat16)
        cps[1].wait()
        o = attention(ln1(x0_ref), 0)
        wo_p[...] = jnp.dot(perm_t, wo_s[...],
                            preferred_element_type=jnp.float32).astype(jnp.bfloat16)
        xn_scr[...] = ln1(x1_ref)
        attention2(x0_ref, o)
        cps[2].wait()
        w1_s[...] = w1t_s[...].T
        cps[3].wait()

    @pl.when(i < nblk - 1)
    def _():
        hn = ln2()
        o = attention(xn_scr[...], i + 1)
        ffn(hn)
        xn_scr[...] = ln1(x2_ref)
        attention2(x1_ref, o)

    @pl.when(i == nblk - 1)
    def _():
        ffn(ln2())


@jax.jit
def pallas_sequential_preLN__sliding_local_dilated__dense_activation_mish__prompt_kernel(
    A_x: jax.Array,
    A_wqkv: jax.Array,
    A_wo: jax.Array,
    B_x: jax.Array,
    B_w1: jax.Array,
    B_b1: jax.Array,
    B_w2: jax.Array,
):
    B, S, D = A_x.shape
    F = B_w1.shape[1]
    tb = 256
    nblk = S // tb
    x = A_x.reshape(B * S, D)
    b1 = B_b1.reshape(1, F)

    const = lambda i: (0, 0)
    hbm = pl.BlockSpec(memory_space=pl.ANY)
    out = pl.pallas_call(
        functools.partial(_kernel, tb=tb, d=D, nblk=nblk),
        grid=(nblk,),
        in_specs=[
            pl.BlockSpec((tb, D), const),
            pl.BlockSpec((tb, D), lambda i: (jnp.minimum(i + 1, nblk - 1), 0)),
            pl.BlockSpec((tb, D), lambda i: (jnp.minimum(i + 2, nblk - 1), 0)),
            hbm,
            hbm,
            hbm,
            pl.BlockSpec((1, F), const),
            hbm,
        ],
        out_specs=pl.BlockSpec((tb, D), lambda i: (i, 0)),
        out_shape=jax.ShapeDtypeStruct((B * S, D), A_x.dtype),
        scratch_shapes=[
            pltpu.VMEM((D, 3 * D), jnp.bfloat16),
            pltpu.VMEM((D, D), jnp.bfloat16),
            pltpu.VMEM((F, D), jnp.bfloat16),
            pltpu.VMEM((F, D), jnp.bfloat16),
            pltpu.VMEM((D, 3 * D), jnp.bfloat16),
            pltpu.VMEM((D, D), jnp.bfloat16),
            pltpu.VMEM((D, F), jnp.bfloat16),
            pltpu.VMEM((tb + HALO, 2 * D), jnp.float32),
            pltpu.VMEM((tb, D), jnp.float32),
            pltpu.VMEM((tb, D), jnp.bfloat16),
            pltpu.SemaphoreType.DMA((4,)),
        ],
        compiler_params=pltpu.CompilerParams(
            dimension_semantics=("arbitrary",),
            vmem_limit_bytes=64 * 1024 * 1024,
        ),
    )(x, x, x, A_wqkv, A_wo, B_w1.T, b1, B_w2)
    return out.reshape(B, S, D)
```
